```python
import os as _os
_os.environ.setdefault("JAX_PLATFORMS", "cpu")
import jax
import jax.numpy as jnp

def _softmax(x, axis=-1):
    return jax.nn.softmax(x, axis=axis)
def _gelu(x):
    return jax.nn.gelu(x, approximate=True)
def _silu(x):
    return jax.nn.silu(x)
def _sigmoid(x):
    return jax.nn.sigmoid(x)
def _layernorm(x, axis=-1, eps=1e-5):
    m = jnp.mean(x, axis=axis, keepdims=True)
    v = jnp.var(x, axis=axis, keepdims=True)
    return (x - m) / jnp.sqrt(v + eps)
def _scatter_add(tgt, idx, src, axis=0):
    return tgt.at[idx].add(src)
def _segment_sum(src, seg, n):
    return jax.ops.segment_sum(src, seg, n)
class _Rng:
    def __init__(self, key):
        self._k = key
    def _next(self):
        self._k, sub = jax.random.split(self._k)
        return sub
    def normal(self, shape):
        return jax.random.normal(self._next(), shape, dtype=jnp.bfloat16)
    def randint(self, lo, hi, shape):
        return jax.random.randint(self._next(), shape, lo, hi, dtype=jnp.int32)
    def uniform(self, shape, lo=0.0, hi=1.0):
        return jax.random.uniform(self._next(), shape, jnp.bfloat16, lo, hi)
    def permutation(self, n):
        return jax.random.permutation(self._next(), n)


kernel_name = 'interleave_layers__sliding_block_cached__mixer_channel_mlp__decode'

def setup_inputs():
    _rng = _Rng(jax.random.key(int.from_bytes(__import__("os").urandom(4), "little")))
    _w = (lambda a: (lambda t: t.astype(jnp.bfloat16) if jnp.issubdtype(t.dtype, jnp.floating) else t)(jnp.asarray(a)))
    def _A_setup():
        B, Sq, D = 8, 1, 1024
        Hq, Hkv, Sk, Dh = 32, 4, 4096, 128
        assert Hq % Hkv == 0, (Hq, Hkv)
        return {
            "x": _w((lambda *s: _rng.normal(s) * 0.05)(B, Sq, D)),
            "k_cache": _w((lambda *s: _rng.normal(s) * 1.6)(B, Hkv, Sk, Dh)),
            "v_cache": _w((lambda *s: _rng.normal(s) * 0.8)(B, Hkv, Sk, Dh)),
            "wq": _w((lambda *s: _rng.normal(s) * 1.6)(D, Hq * Dh) * (D ** -0.5)),
            "wo": _w((lambda *s: _rng.normal(s) * 0.8)(Hq * Dh, D) * ((Hq * Dh) ** -0.5)),
        }
    _A_in = _A_setup()

    def _B_setup():
        B, S, D, F = 8, 1, 1024, 3584
        return {
            "x": _w((lambda *s: _rng.normal(s) * 0.05)(B, S, D)),
            "w1": _w((lambda *s: _rng.normal(s) * 0.4)(D, F) * (D ** -0.5)),
            "b1": _w((lambda *s: _rng.normal(s) * 0.4)(F)),
            "w2": _w((lambda *s: _rng.normal(s) * 0.4)(F, D) * (F ** -0.5)),
            "b2": _w((lambda *s: _rng.normal(s) * 0.1)(D)),
        }
    _B_in = _B_setup()

    return {
        "A_x": _A_in["x"],
        "A_k_cache": _A_in["k_cache"],
        "A_v_cache": _A_in["v_cache"],
        "A_wq": _A_in["wq"],
        "A_wo": _A_in["wo"],
        "B_x": _B_in["x"],
        "B_w1": _B_in["w1"],
        "B_b1": _B_in["b1"],
        "B_w2": _B_in["w2"],
        "B_b2": _B_in["b2"],
    }

def reference(A_x, A_k_cache, A_v_cache, A_wq, A_wo, B_x, B_w1, B_b1, B_w2, B_b2):
    def _A_ref(x, k_cache, v_cache, wq, wo):
        B, Sq, D = x.shape
        Hq, Dh = 32, 128
        Hkv, Sk = k_cache.shape[1], k_cache.shape[2]
        W = min(4096, max(256, Sk // 4))
        rep = Hq // Hkv
        q = (lambda x, *d: x.transpose(*d))((x @ wq).reshape(B, Sq, Hq, Dh), 0, 2, 1, 3)
        k = jnp.repeat(k_cache[:, :, Sk - W:, :], rep, axis=1)
        v = jnp.repeat(v_cache[:, :, Sk - W:, :], rep, axis=1)
        scores = jnp.einsum("bhqd,bhkd->bhqk", q, k) * (Dh ** -0.5)
        p = _softmax(scores, axis=-1)
        o = jnp.einsum("bhqk,bhkd->bhqd", p, v)
        return (lambda x, *d: x.transpose(*d))(o, 0, 2, 1, 3).reshape(B, Sq, Hq * Dh) @ wo

    def _B_ref(x, w1, b1, w2, b2):
        y = _layernorm(x, axis=-1)
        h = _gelu(jnp.einsum("bsd,df->bsf", y, w1) + b1)
        return jnp.einsum("bsf,fd->bsd", h, w2) + b2

    x = A_x
    x = x + _A_ref(_layernorm(x, axis=-1), A_k_cache, A_v_cache, A_wq, A_wo)
    x = x + _B_ref(_layernorm(x, axis=-1), B_w1, B_b1, B_w2, B_b2)
    x = x + _A_ref(_layernorm(x, axis=-1), A_k_cache, A_v_cache, A_wq, A_wo)
    x = x + _B_ref(_layernorm(x, axis=-1), B_w1, B_b1, B_w2, B_b2)
    return x
```

```python
import functools
import numpy as np
import jax
import jax.numpy as jnp
from jax import lax
import jax.experimental.pallas as pl
import jax.experimental.pallas.tpu as pltpu

B, D, HQ, HKV, DH, F = 8, 1024, 32, 4, 128, 3584
REP = HQ // HKV
EPS = 1e-5
BF, F32, U32 = jnp.bfloat16, jnp.float32, jnp.uint32


def _tiles(w):
    k, n = w.shape
    return w.reshape(k // 16, 2, 8, n // 128, 128).transpose(0, 1, 3, 2, 4)


def _ln(x):
    m = jnp.mean(x, axis=-1, keepdims=True)
    c = x - m
    v = jnp.mean(c * c, axis=-1, keepdims=True)
    return c * lax.rsqrt(v + EPS)


def _gelu(x):
    return 0.5 * x * (1.0 + jnp.tanh(np.float32(np.sqrt(2 / np.pi)) * (x + 0.044715 * (x * x * x))))


def _w(ref32, k0, nk, j0, nj):
    cols = []
    for j in range(j0, j0 + nj):
        t = ref32[pl.ds(k0 // 16, nk // 16), j]
        cols.append(pltpu.bitcast(t.reshape(nk // 2, 128), BF))
    return cols[0] if nj == 1 else jnp.concatenate(cols, axis=1)


def _dot(a, b):
    return jnp.dot(a, b, preferred_element_type=F32)


def make(window=4, nsem=8, wq_rows=128, wo_rows=512, w1_rows=128, w2_chunks=(512,) * 6 + (256, 128, 128), cp=None):
    def kernel(x_hbm, k_hbm, v_hbm, wq_hbm, wo_hbm, w1_hbm, b1_hbm, w2_hbm, b2_hbm, o_hbm,
               xb, b1b, b2b, ob, kb, kt, vb, wqb, wob, w1b, w2b, qs, os_, ps, ls, sems, ssem):
        SK = k_hbm.shape[2]
        W = kb.shape[2]
        NS = W // 128
        wq32, wo32, w132, w232, v32 = (r.bitcast(U32) for r in (wqb, wob, w1b, w2b, vb))

        groups = []

        def add_w(src, dst, k0, nk):
            s = sems.at[len(groups) % nsem]
            groups.append([pltpu.make_async_copy(src.at[pl.ds(k0 // 16, nk // 16), h],
                                                 dst.at[pl.ds(k0 // 16, nk // 16), :, pl.ds(8 * h, 8), :], s)
                           for h in range(2)])

        def add_kv(src, dst, b):
            s = sems.at[len(groups) % nsem]
            groups.append([pltpu.make_async_copy(src.at[b, :, pl.ds(SK - W, W), :], dst.at[b], s)])

        for k0 in range(0, D, wq_rows): add_w(wq_hbm, wqb, k0, wq_rows)
        for b in range(B): add_kv(k_hbm, kb, b)
        for b in range(B): add_kv(v_hbm, vb, b)
        for k0 in range(0, HQ * DH, wo_rows): add_w(wo_hbm, wob, k0, wo_rows)
        for k0 in range(0, D, w1_rows): add_w(w1_hbm, w1b, k0, w1_rows)
        k0 = 0
        for nk in w2_chunks:
            add_w(w2_hbm, w2b, k0, nk)
            k0 += nk
        assert k0 == F
        n = len(groups)
        small = [pltpu.make_async_copy(s, d, ssem.at[i]) for i, (s, d) in enumerate(((x_hbm, xb), (b1_hbm, b1b), (b2_hbm, b2b)))]
        for c in groups[0]: c.start()
        for c in small: c.start()
        for g in groups[1:window]:
            for c in g: c.start()
        pos = [0]

        def arrive():
            i = pos[0]
            pos[0] += 1
            for c in groups[i]: c.wait()
            if i + window < n:
                for c in groups[i + window]: c.start()

        qscale = np.float32(DH ** -0.5 * np.log2(np.e))

        def put_q(q, h0):
            for i in range(q.shape[1] // DH):
                qs[pl.ds((h0 + i) * B, B), :] = q[:, i * DH:(i + 1) * DH] * qscale

        def scores(b, g):
            q = qs[pl.ds(g * REP * B + b, REP, stride=B), :].astype(BF)
            kk = jnp.concatenate([pltpu.bitcast(kt[b, g, j], BF) for j in range(NS)], axis=1)
            s = _dot(q, kk)
            p = jnp.exp2(s - jnp.max(s, axis=-1, keepdims=True))
            return p.astype(BF), 1.0 / jnp.sum(p, axis=-1, keepdims=True)

        def pv(b, g, p, rl):
            o = _dot(p, pltpu.bitcast(v32[b, g], BF)) * rl
            os_[pl.ds((g * B + b) * REP, REP), :] = o

        def o_rows(h0, nh):
            return jnp.concatenate(
                [os_[pl.ds((h // REP) * B * REP + h % REP, B, stride=REP), :] for h in range(h0, h0 + nh)],
                axis=1).astype(BF)

        for c in small: c.wait()
        x = xb[...].astype(F32)
        b1 = b1b[...].astype(F32)
        b2f = b2b[...].astype(F32)
        b2 = jnp.concatenate([jnp.broadcast_to(b2f[j:j + 1], (B, 128)) for j in range(D // 128)], axis=1)
        b1 = jnp.concatenate([jnp.broadcast_to(b1[j:j + 1], (B, 128)) for j in range(F // 128)], axis=1)
        y = _ln(x).astype(BF)
        q = None
        for k0 in range(0, D, wq_rows):
            arrive()
            d = _dot(y[:, k0:k0 + wq_rows], _w(wq32, k0, wq_rows, 0, HQ))
            q = d if q is None else q + d
        put_q(q, 0)
        for b in range(B):
            arrive()
            for g in range(HKV):
                for j in range(NS):
                    kt[b, g, j] = pltpu.bitcast(kb[b, g, pl.ds(j * 128, 128), :].T, U32)
                p, rl = scores(b, g)
                ps[b, g] = p.astype(F32)
                ls[b, g] = jnp.broadcast_to(rl, (REP, 128))
        for b in range(B):
            arrive()
            for g in range(HKV):
                pv(b, g, ps[b, g].astype(BF), ls[b, g])
        for k0 in range(0, HQ * DH, wo_rows):
            arrive()
            x = x + _dot(o_rows(k0 // DH, wo_rows // DH), _w(wo32, k0, wo_rows, 0, D // 128))
        y = _ln(_ln(x)).astype(BF)
        h = b1
        for k0 in range(0, D, w1_rows):
            arrive()
            h = h + _dot(y[:, k0:k0 + w1_rows], _w(w132, k0, w1_rows, 0, F // 128))
        h = _gelu(h).astype(BF)
        x = x + b2
        k0 = 0
        for nk in w2_chunks:
            arrive()
            x = x + _dot(h[:, k0:k0 + nk], _w(w232, k0, nk, 0, D // 128))
            k0 += nk
        assert pos[0] == n

        y = _ln(x).astype(BF)
        for g in range(HKV):
            put_q(_dot(y, _w(wq32, 0, D, g * REP, REP)), g * REP)
        for g in range(HKV):
            pr = [scores(b, g) for b in range(B)]
            for b in range(B):
                pv(b, g, *pr[b])
        for g in range(HKV):
            x = x + _dot(o_rows(g * REP, REP), _w(wo32, g * REP * DH, REP * DH, 0, D // 128))
        y = _ln(_ln(x)).astype(BF)
        FC = 512
        hs = [_gelu(b1[:, f0:f0 + FC] + _dot(y, _w(w132, 0, D, f0 // 128, FC // 128))).astype(BF) for f0 in range(0, F, FC)]
        x = x + b2
        for i, f0 in enumerate(range(0, F, FC)):
            x = x + _dot(hs[i], _w(w232, f0, FC, 0, D // 128))
        ob[...] = x.astype(ob.dtype)
        c = pltpu.make_async_copy(ob, o_hbm, ssem.at[0])
        c.start()
        c.wait()

    def fn(A_x, A_k_cache, A_v_cache, A_wq, A_wo, B_x, B_w1, B_b1, B_w2, B_b2):
        sk = A_k_cache.shape[2]
        w = min(4096, max(256, sk // 4))
        out = pl.pallas_call(
            kernel,
            out_shape=jax.ShapeDtypeStruct((B, D), A_x.dtype),
            in_specs=[pl.BlockSpec(memory_space=pl.ANY)] * 9,
            out_specs=pl.BlockSpec(memory_space=pl.ANY),
            scratch_shapes=[
                pltpu.VMEM((B, D), BF), pltpu.VMEM((F // 128, 128), BF), pltpu.VMEM((D // 128, 128), BF),
                pltpu.VMEM((B, D), A_x.dtype),
                pltpu.VMEM((B, HKV, w, DH), BF), pltpu.VMEM((B, HKV, w // 128, DH // 2, 128), U32),
                pltpu.VMEM((B, HKV, w, DH), BF),
                pltpu.VMEM((D // 16, HQ, 16, 128), BF), pltpu.VMEM((HQ * DH // 16, D // 128, 16, 128), BF),
                pltpu.VMEM((D // 16, F // 128, 16, 128), BF), pltpu.VMEM((F // 16, D // 128, 16, 128), BF),
                pltpu.VMEM((HQ * B, DH), F32), pltpu.VMEM((HQ * B, DH), F32),
                pltpu.VMEM((B, HKV, REP, w), F32), pltpu.VMEM((B, HKV, REP, 128), F32),
                pltpu.SemaphoreType.DMA((nsem,)), pltpu.SemaphoreType.DMA((3,)),
            ],
            compiler_params=pltpu.CompilerParams(vmem_limit_bytes=100 * 1024 * 1024, **(cp or {})),
        )(A_x.reshape(B, D), A_k_cache, A_v_cache, _tiles(A_wq), _tiles(A_wo), _tiles(B_w1),
          B_b1.reshape(F // 128, 128), _tiles(B_w2), B_b2.reshape(D // 128, 128))
        return out.reshape(A_x.shape)
    return fn


@jax.jit
def pallas_interleave_layers__sliding_block_cached__mixer_channel_mlp__decode_kernel(
    A_x, A_k_cache, A_v_cache, A_wq, A_wo, B_x, B_w1, B_b1, B_w2, B_b2
):
    return make()(A_x, A_k_cache, A_v_cache, A_wq, A_wo, B_x, B_w1, B_b1, B_w2, B_b2)
```

```python
import numpy as np
import jax
import jax.numpy as jnp
from jax import lax
import jax.experimental.pallas as pl
import jax.experimental.pallas.tpu as pltpu

B, D, HQ, HKV, DH, F, W = 8, 1024, 32, 4, 128, 3584, 1024
REP = HQ // HKV
ND, NF, NS = D // 128, F // 128, W // 128
GW = REP * DH
EPS = 1e-5
BF, F32, U32 = jnp.bfloat16, jnp.float32, jnp.uint32

WQ_PIECES = [(k, 2, 0, HQ) for k in range(0, ND, 2)]
WO_PIECES = [(k, REP, 0, ND) for k in range(0, HQ, REP)]
W1_PIECES = [(k, 2, 0, NF) for k in range(0, ND, 2)]
W2_GROUPS = [
    [(0, 16, 0, 5), (16, 12, 0, 5)],
    [(0, 20, 5, 2), (20, 8, 5, 2)],
    [(0, 16, 7, 1), (16, 8, 7, 1), (24, 4, 7, 1)],
]
W2_PIECES = [p for group in W2_GROUPS for p in group]
IN_FLIGHT = 3

VPU_PV = (7, 0)
VPU_WO = [(8, 16, 7)]
VPU_W2 = [(0, 8, 0), (8, 12, 1)]
VPU_CHAINS = 2
LAGS = (2, 4, 8)
STEP_WO, STEP_W2 = 2, 4


def _tile_view(w):
    k, n = w.shape
    return w.reshape(k // 16, 2, 8, n // 128, 128).transpose(0, 1, 3, 2, 4)


def _piece_scratch(pieces):
    return [pltpu.VMEM((nk * 8, nj, 16, 128), BF) for _, nk, _, nj in pieces]


def _dot(a, b):
    return jnp.dot(a, b, preferred_element_type=F32)


def _blk(x, j, n=1):
    return x[:, j * 128:(j + n) * 128]


def _cat(xs):
    return xs[0] if len(xs) == 1 else jnp.concatenate(xs, axis=1)


def _mean(x):
    return jnp.mean(x, axis=-1, keepdims=True)


def _moments(x):
    m = _mean(x)
    c = x - m
    return m, c, lax.rsqrt(_mean(c * c) + EPS)


def _layernorm(x):
    _, c, r = _moments(x)
    return c * r


def _gelu(x):
    return 0.5 * x * (1.0 + jnp.tanh(np.float32(np.sqrt(2 / np.pi)) * (x + 0.044715 * (x * x * x))))


def _with_ones(y):
    return jnp.concatenate([y, jnp.ones_like(y)], axis=0).astype(BF)


def _rows_to_lanes(b):
    b = b.astype(F32)
    return _cat([jnp.broadcast_to(b[j:j + 1], (B, 128)) for j in range(b.shape[0])])


class _Weight:
    def __init__(self, pieces, refs):
        self.pieces = pieces
        self.words = [r.bitcast(U32) for r in refs]

    def column(self, k, nk, j, piece_j=None):
        parts = []
        for (k0, pk, j0, pj), ref in sorted(zip(self.pieces, self.words), key=lambda t: t[0]):
            lo, hi = max(k, k0), min(k + nk, k0 + pk)
            if lo < hi and j0 <= (j if piece_j is None else piece_j) < j0 + pj:
                t = ref[pl.ds((lo - k0) * 8, (hi - lo) * 8), j - j0]
                parts.append(pltpu.bitcast(t.reshape((hi - lo) * 64, 128), BF))
        return parts[0] if len(parts) == 1 else jnp.concatenate(parts, axis=0)

    def block(self, k, nk, js, piece_j=None):
        return _cat([self.column(k, nk, j, piece_j) for j in js])


def _kernel(x_hbm, k_hbm, v_hbm, wq_hbm, wo_hbm, w1_hbm, b1_hbm, w2_hbm, b2_hbm, out_hbm,
            x_buf, b1_buf, b2_buf, out_buf, k_bufs, v_bufs, wq_bufs, wo_bufs, w1_bufs, w2_bufs,
            kt, q_heads, o_heads, probs, wq_sum, w1_sum, q_part, pv_t, wo_t, w2_t, zeros, sems):
    wq, wo = _Weight(WQ_PIECES, wq_bufs), _Weight(WO_PIECES, wo_bufs)
    w1, w2 = _Weight(W1_PIECES, w1_bufs), _Weight(W2_PIECES, w2_bufs)
    v_words = [r.bitcast(U32) for r in v_bufs]
    window = pl.ds(k_hbm.shape[2] - W, W)

    def weight_copies(src, pieces, bufs):
        return [[(src.at[pl.ds(k * 8, nk * 8), h, pl.ds(j, nj)], buf.at[:, :, pl.ds(h * 8, 8), :])
                 for h in range(2)] for (k, nk, j, nj), buf in zip(pieces, bufs)]

    plan = [[(x_hbm, x_buf), (b1_hbm, b1_buf), (b2_hbm, b2_buf)]]
    plan += weight_copies(wq_hbm, WQ_PIECES, wq_bufs)
    plan += [[(k_hbm.at[b, :, window, :], k_bufs[b])] for b in range(B)]
    plan += [[(v_hbm.at[b, :, window, :], v_bufs[b])] for b in range(B)]
    plan += weight_copies(wo_hbm, WO_PIECES, wo_bufs)
    plan += weight_copies(w1_hbm, W1_PIECES, w1_bufs)
    plan += weight_copies(w2_hbm, W2_PIECES, w2_bufs)
    copies = [[pltpu.make_async_copy(src, dst, sems.at[i % IN_FLIGHT]) for src, dst in step]
              for i, step in enumerate(plan)]
    for step in copies[:IN_FLIGHT]:
        for c in step:
            c.start()
    landed = []

    def next_piece():
        i = len(landed)
        landed.append(i)
        for c in copies[i]:
            c.wait()
        for step in copies[i + IN_FLIGHT:i + IN_FLIGHT + 1]:
            for c in step:
                c.start()

    q_scale = np.float32(DH ** -0.5 * np.log2(np.e))

    def put_q(g, q):
        for i in range(REP):
            q_heads[g][pl.ds(i * B, B), :] = _blk(q, i)

    def logits(b, g):
        q = q_heads[g][pl.ds(b, REP, stride=B), :].astype(BF)
        return _dot(q, _cat([pltpu.bitcast(kt[b, g, j], BF) for j in range(NS)]))

    def row_max(s):
        return jnp.max(s, axis=-1, keepdims=True)

    def softmax(s, top):
        p = jnp.exp2(s - top)
        return p * (1.0 / jnp.sum(p, axis=-1, keepdims=True))

    def put_o(b, g, o):
        o_heads[g][pl.ds(b * REP, REP), :] = o

    def p_times_v(b, g, p):
        put_o(b, g, _dot(p.astype(BF), pltpu.bitcast(v_words[b][g], BF)))

    def get_o(g):
        return _cat([o_heads[g][pl.ds(i, B, stride=REP), :] for i in range(REP)])

    def stage(dst, tiles):
        for i, t in enumerate(tiles):
            t = t.astype(F32).T
            dst[i, pl.ds(0, 128), :] = t
            dst[i, pl.ds(128, 8), :] = t[:8]

    def stage_weight(w, jobs, dsts, piece):
        k0, pk, j0, pj = piece
        for (k, nk, j), dst in zip(jobs, dsts):
            if k0 < k + nk <= k0 + pk and j0 <= j < j0 + pj:
                stage(dst, [w.column(k + i, 1, j) for i in range(nk)])

    zeros[...] = jnp.zeros_like(zeros)
    next_piece()
    x = x_buf[...].astype(F32)
    b1, b2 = _rows_to_lanes(b1_buf[...]), _rows_to_lanes(b2_buf[...])

    y = _with_ones(_layernorm(x))
    q = None
    for k, nk, _, _ in WQ_PIECES:
        next_piece()
        d = _dot(_blk(y, k, nk), wq.block(k, nk, range(HQ)))
        q = d if q is None else q + d
    for g in range(HKV):
        put_q(g, _blk(q[:B], g * REP, REP) * q_scale)
    wq_sum[...] = q[B:]
    for b in range(B):
        next_piece()
        for g in range(HKV):
            for j in range(NS):
                kt[b, g, j] = pltpu.bitcast(k_bufs[b][g, pl.ds(j * 128, 128), :].T, U32)
            s = logits(b, g)
            probs[b, g] = softmax(s, row_max(s))
    for b in range(B):
        next_piece()
        for g in range(HKV):
            p_times_v(b, g, probs[b, g])
        if b == VPU_PV[0]:
            stage(pv_t, [v_bufs[b][VPU_PV[1], pl.ds(i * 128, 128), :] for i in range(NS)])
    for g, piece in enumerate(WO_PIECES):
        next_piece()
        x = x + _dot(get_o(g).astype(BF), wo.block(g * REP, REP, range(ND)))
        stage_weight(wo, VPU_WO, wo_t, piece)

    y = _with_ones(_layernorm(_layernorm(x)))
    h = None
    for k, nk, _, _ in W1_PIECES:
        next_piece()
        d = _dot(_blk(y, k, nk), w1.block(k, nk, range(NF)))
        h = d if h is None else h + d
    w1_sum[...] = h[B:]
    h = _gelu(h[:B] + b1).astype(BF)
    x = x + b2

    def finish_columns(group):
        _, _, j, nj = group[0]
        xj = _blk(x, j, nj)
        for piece in group:
            k, nk, _, _ = piece
            next_piece()
            xj = xj + _dot(_blk(h, k, nk), w2.block(k, nk, range(j, j + nj)))
            stage_weight(w2, VPU_W2, w2_t, piece)
        return j, nj, xj.astype(BF)

    early = []
    for group in W2_GROUPS[:-1]:
        j, nj, xj = finish_columns(group)

        def q_share(i, carry, j=j, nj=nj, xj=xj):
            d = _dot(xj, wq.block(j, nj, [i * (HQ // 2) + c for c in range(HQ // 2)], piece_j=0))
            q_part[i] = d if j == 0 else q_part[i] + d
            return carry

        lax.fori_loop(0, 2, q_share, None)
        early.append(xj.astype(F32))
    early = _cat(early)
    shift = _mean(early)
    c = early - shift
    sum1, sum2 = jnp.sum(c, axis=-1, keepdims=True), jnp.sum(c * c, axis=-1, keepdims=True)
    j, nj, late = finish_columns(W2_GROUPS[-1])
    assert len(landed) == len(copies)
    c = late.astype(F32) - shift
    dm = (sum1 + jnp.sum(c, axis=-1, keepdims=True)) * (1.0 / D)
    var = (sum2 + jnp.sum(c * c, axis=-1, keepdims=True)) * (1.0 / D) - dm * dm
    mean, mul = shift + dm, lax.rsqrt(jnp.maximum(var, 0.0) + EPS) * q_scale
    x = _cat([early, late.astype(F32)])

    never = zeros[...] != 0
    diagonal = (lax.broadcasted_iota(jnp.int32, (B, 128), 1)
                - lax.broadcasted_iota(jnp.int32, (B, 128), 0)) & 127
    chains = [None] * VPU_CHAINS

    def vpu_matmul(a, wt):
        out = jnp.zeros((B, 128), F32)
        for s in range(128):
            t = _blk(a, 0) * wt[0, pl.ds(s, 8), :]
            if chains[s % VPU_CHAINS] is not None:
                t = jnp.where(never, chains[s % VPU_CHAINS], t)
            for i in range(1, wt.shape[0]):
                t = t + _blk(a, i) * wt[i, pl.ds(s, 8), :]
            chains[s % VPU_CHAINS] = t
            out = jnp.where(diagonal == s, jnp.sum(t, axis=-1, keepdims=True), out)
        return out

    def add_matmul(x, blocks, w, jobs, staged, step):
        acc = [_blk(x, j) for j in range(ND)]
        for k in range(0, len(blocks), step):
            js = [j for j in range(ND) if not any(k0 <= k < k0 + nk and j == j0 for k0, nk, j0 in jobs)]
            d = _dot(_cat(blocks[k:k + step]).astype(BF), w.block(k, step, js))
            for i, j in enumerate(js):
                acc[j] = acc[j] + _blk(d, i)
        for (k, nk, j), wt in zip(jobs, staged):
            assert k % step == 0 and nk % step == 0
            acc[j] = acc[j] + vpu_matmul(_cat(blocks[k:k + nk]), wt)
        return _cat(acc)

    for g in range(HKV):
        q = q_part[g // 2, :, pl.ds(g % 2 * GW, GW)] + _dot(late, wq.block(j, nj, range(g * REP, (g + 1) * REP)))
        put_q(g, (q - mean * wq_sum[:, pl.ds(g * GW, GW)]) * mul)
    pairs = [(b, g) for g in range(HKV) for b in range(B)]
    s, top, p = {}, {}, {}
    for i in range(len(pairs) + LAGS[2]):
        now, at_max, at_exp, at_pv = (pairs[i - n] if 0 <= i - n < len(pairs) else None for n in (0,) + LAGS)
        if now:
            s[now] = logits(*now)
        if at_max:
            top[at_max] = row_max(s[at_max])
        if at_exp:
            p[at_exp] = softmax(s[at_exp], top[at_exp])
        if at_pv == VPU_PV:
            put_o(*at_pv, vpu_matmul(p[at_pv], pv_t))
        elif at_pv:
            p_times_v(*at_pv, p[at_pv])
    o = [get_o(g) for g in range(HKV)]
    x = add_matmul(x, [_blk(o[i // REP], i % REP) for i in range(HQ)], wo, VPU_WO, wo_t, STEP_WO)

    xr = x.astype(BF)
    m1, c, r1 = _moments(xr.astype(F32))
    m2, _, r2 = _moments(c * r1)
    mul, sub = r1 * r2, (m1 * r1 + m2) * r2
    h = [_gelu(_dot(xr, w1.column(0, ND, f)) * mul - sub * w1_sum[:, pl.ds(f * 128, 128)] + _blk(b1, f))
         for f in range(NF)]
    x = add_matmul(x + b2, h, w2, VPU_W2, w2_t, STEP_W2)

    out_buf[...] = x.astype(out_buf.dtype)
    copy_out = pltpu.make_async_copy(out_buf, out_hbm, sems.at[0])
    copy_out.start()
    copy_out.wait()


@jax.jit
def pallas_interleave_layers__sliding_block_cached__mixer_channel_mlp__decode_kernel(
    A_x: jax.Array,
    A_k_cache: jax.Array,
    A_v_cache: jax.Array,
    A_wq: jax.Array,
    A_wo: jax.Array,
    B_x: jax.Array,
    B_w1: jax.Array,
    B_b1: jax.Array,
    B_w2: jax.Array,
    B_b2: jax.Array,
):
    del B_x
    sk = A_k_cache.shape[2]
    assert A_x.shape == (B, 1, D) and A_k_cache.shape == A_v_cache.shape == (B, HKV, sk, DH)
    assert min(4096, max(256, sk // 4)) == W and B_w1.shape == (D, F)
    staged = lambda nk: pltpu.VMEM((nk, 136, 128), F32)
    out = pl.pallas_call(
        _kernel,
        out_shape=jax.ShapeDtypeStruct((B, D), A_x.dtype),
        in_specs=[pl.BlockSpec(memory_space=pl.ANY)] * 9,
        out_specs=pl.BlockSpec(memory_space=pl.ANY),
        scratch_shapes=[
            pltpu.VMEM((B, D), BF),
            pltpu.VMEM((NF, 128), BF),
            pltpu.VMEM((ND, 128), BF),
            pltpu.VMEM((B, D), A_x.dtype),
            [pltpu.VMEM((HKV, W, DH), BF)] * B,
            [pltpu.VMEM((HKV, W, DH), BF)] * B,
            _piece_scratch(WQ_PIECES),
            _piece_scratch(WO_PIECES),
            _piece_scratch(W1_PIECES),
            _piece_scratch(W2_PIECES),
            pltpu.VMEM((B, HKV, NS, DH // 2, 128), U32),
            [pltpu.VMEM((REP * B, DH), F32)] * HKV,
            [pltpu.VMEM((B * REP, DH), F32)] * HKV,
            pltpu.VMEM((B, HKV, REP, W), F32),
            pltpu.VMEM((B, HQ * DH), F32),
            pltpu.VMEM((B, F), F32),
            pltpu.VMEM((2, B, HQ * DH // 2), F32),
            staged(NS),
            [staged(nk) for _, nk, _ in VPU_WO],
            [staged(nk) for _, nk, _ in VPU_W2],
            pltpu.VMEM((B, 128), jnp.int32),
            pltpu.SemaphoreType.DMA((IN_FLIGHT,)),
        ],
        compiler_params=pltpu.CompilerParams(vmem_limit_bytes=80 * 1024 * 1024),
    )(
        A_x.reshape(B, D), A_k_cache, A_v_cache, _tile_view(A_wq), _tile_view(A_wo), _tile_view(B_w1),
        B_b1.reshape(NF, 128), _tile_view(B_w2), B_b2.reshape(ND, 128),
    )
    return out.reshape(A_x.shape)
```

```python
import numpy as np
import jax
import jax.numpy as jnp
from jax import lax
import jax.experimental.pallas as pl
import jax.experimental.pallas.tpu as pltpu

B, D, HQ, HKV, DH, F, W = 8, 1024, 32, 4, 128, 3584, 1024
REP = HQ // HKV
ND, NF, NS = D // 128, F // 128, W // 128
GW = REP * DH
EPS = 1e-5
BF, F32, U32 = jnp.bfloat16, jnp.float32, jnp.uint32

WO_PIECES = [(k, REP, 0, ND) for k in range(0, HQ, REP)]
W1_PIECES = [(k, 2, 0, NF) for k in range(0, ND, 2)]
W2_GROUPS = [
    [(0, 16, 0, 5), (16, 12, 0, 5)],
    [(0, 20, 5, 2), (20, 8, 5, 2)],
    [(0, 16, 7, 1), (16, 8, 7, 1), (24, 4, 7, 1)],
]
W2_PIECES = [p for group in W2_GROUPS for p in group]
WQ_PIECES = [group[0][2:] + (0, HQ) for group in W2_GROUPS]
IN_FLIGHT = 3

VPU_PV = (7, 0)
VPU_WO = [(8, 16, 7)]
VPU_W2 = [(0, 8, 0), (8, 12, 1)]
VPU_CHAINS = 2
LAGS = (2, 4, 8)
STEP_WO, STEP_W2 = 2, 4


def _landing_scratch(pieces):
    return [pltpu.VMEM((nk * 128, nj * 128), BF) for _, nk, _, nj in pieces]


def _packed_scratch(pieces):
    return [pltpu.VMEM((nk * 64, nj * 128), U32) for _, nk, _, nj in pieces]


def _dot(a, b):
    return jnp.dot(a, b, preferred_element_type=F32)


def _blk(x, j, n=1):
    return x[:, j * 128:(j + n) * 128]


def _cat(xs):
    return xs[0] if len(xs) == 1 else jnp.concatenate(xs, axis=1)


def _mean(x):
    return jnp.mean(x, axis=-1, keepdims=True)


def _moments(x):
    m = _mean(x)
    c = x - m
    return m, c, lax.rsqrt(_mean(c * c) + EPS)


def _layernorm(x):
    _, c, r = _moments(x)
    return c * r


def _gelu(x):
    return 0.5 * x * (1.0 + jnp.tanh(np.float32(np.sqrt(2 / np.pi)) * (x + 0.044715 * (x * x * x))))


def _with_ones(y):
    return jnp.concatenate([y, jnp.ones_like(y)], axis=0).astype(BF)


def _rows_to_lanes(b):
    b = b.astype(F32)
    return _cat([jnp.broadcast_to(b[j:j + 1], (B, 128)) for j in range(b.shape[0])])


class _Weight:
    def __init__(self, pieces, landing, packed):
        self.pieces, self.landing, self.packed = pieces, landing, packed

    def first_read(self, piece):
        i = self.pieces.index(piece)
        w = self.landing[i][...]
        self.packed[i][...] = pltpu.bitcast(w, U32)
        return w

    def column(self, k, nk, j):
        parts = []
        for (k0, pk, j0, pj), ref in zip(self.pieces, self.packed):
            lo, hi = max(k, k0), min(k + nk, k0 + pk)
            if lo < hi and j0 <= j < j0 + pj:
                t = ref[pl.ds((lo - k0) * 64, (hi - lo) * 64), pl.ds((j - j0) * 128, 128)]
                parts.append(pltpu.bitcast(t, BF))
        return parts[0] if len(parts) == 1 else jnp.concatenate(parts, axis=0)

    def block(self, k, nk, js):
        return _cat([self.column(k, nk, j) for j in js])


def _kernel(x_hbm, k_hbm, v_hbm, wq_hbm, wo_hbm, w1_hbm, b1_hbm, w2_hbm, b2_hbm, out_hbm,
            x_buf, b1_buf, b2_buf, out_buf, k_bufs, v_bufs, wq_bufs, wo_bufs, w1_bufs, w2_bufs,
            kt, v_packed, wq_packed, wo_packed, w1_packed, w2_packed,
            q_heads, o_heads, probs, wq_sum, w1_sum, q_part, pv_t, wo_t, w2_t, zeros, sems):
    wq, wo = _Weight(WQ_PIECES, wq_bufs, wq_packed), _Weight(WO_PIECES, wo_bufs, wo_packed)
    w1, w2 = _Weight(W1_PIECES, w1_bufs, w1_packed), _Weight(W2_PIECES, w2_bufs, w2_packed)
    window = pl.ds(k_hbm.shape[2] - W, W)

    def weight_copies(src, pieces, bufs):
        return [[(src.at[pl.ds(k * 128, nk * 128), pl.ds(j * 128, nj * 128)], buf)]
                for (k, nk, j, nj), buf in zip(pieces, bufs)]

    plan = [[(x_hbm, x_buf), (b1_hbm, b1_buf), (b2_hbm, b2_buf)]]
    plan += weight_copies(wq_hbm, WQ_PIECES, wq_bufs)
    plan += [[(k_hbm.at[b, :, window, :], k_bufs[b])] for b in range(B)]
    plan += [[(v_hbm.at[b, :, window, :], v_bufs[b])] for b in range(B)]
    plan += weight_copies(wo_hbm, WO_PIECES, wo_bufs)
    plan += weight_copies(w1_hbm, W1_PIECES, w1_bufs)
    plan += weight_copies(w2_hbm, W2_PIECES, w2_bufs)
    copies = [[pltpu.make_async_copy(src, dst, sems.at[i % IN_FLIGHT]) for src, dst in step]
              for i, step in enumerate(plan)]
    for step in copies[:IN_FLIGHT]:
        for c in step:
            c.start()
    landed = []

    def next_piece():
        i = len(landed)
        landed.append(i)
        for c in copies[i]:
            c.wait()
        for step in copies[i + IN_FLIGHT:i + IN_FLIGHT + 1]:
            for c in step:
                c.start()

    q_scale = np.float32(DH ** -0.5 * np.log2(np.e))

    def put_q(g, q):
        for i in range(REP):
            q_heads[g][pl.ds(i * B, B), :] = _blk(q, i)

    def logits(b, g):
        q = q_heads[g][pl.ds(b, REP, stride=B), :].astype(BF)
        return _dot(q, _cat([pltpu.bitcast(kt[b, g, j], BF) for j in range(NS)]))

    def row_max(s):
        return jnp.max(s, axis=-1, keepdims=True)

    def softmax(s, top):
        p = jnp.exp2(s - top)
        return p * (1.0 / jnp.sum(p, axis=-1, keepdims=True))

    def put_o(b, g, o):
        o_heads[g][pl.ds(b * REP, REP), :] = o

    def get_o(g):
        return _cat([o_heads[g][pl.ds(i, B, stride=REP), :] for i in range(REP)])

    def stage(dst, tiles):
        for i, t in enumerate(tiles):
            t = t.astype(F32).T
            dst[i, pl.ds(0, 128), :] = t
            dst[i, pl.ds(128, 8), :] = t[:8]

    def stage_weight(w, jobs, dsts, piece):
        k0, pk, j0, pj = piece
        for (k, nk, j), dst in zip(jobs, dsts):
            if k0 < k + nk <= k0 + pk and j0 <= j < j0 + pj:
                stage(dst, [w.column(k + i, 1, j) for i in range(nk)])

    zeros[...] = jnp.zeros_like(zeros)
    next_piece()
    x = x_buf[...].astype(F32)
    b1, b2 = _rows_to_lanes(b1_buf[...]), _rows_to_lanes(b2_buf[...])

    y = _with_ones(_layernorm(x))
    q = None
    for piece in WQ_PIECES:
        next_piece()
        d = _dot(_blk(y, *piece[:2]), wq.first_read(piece))
        q = d if q is None else q + d
    for g in range(HKV):
        put_q(g, _blk(q[:B], g * REP, REP) * q_scale)
    wq_sum[...] = q[B:]
    for b in range(B):
        next_piece()
        for g in range(HKV):
            for j in range(NS):
                kt[b, g, j] = pltpu.bitcast(k_bufs[b][g, pl.ds(j * 128, 128), :].T, U32)
            s = logits(b, g)
            probs[b, g] = softmax(s, row_max(s))
    for b in range(B):
        next_piece()
        for g in range(HKV):
            v = v_bufs[b][g]
            v_packed[b, g] = pltpu.bitcast(v, U32)
            put_o(b, g, _dot(probs[b, g].astype(BF), v))
        if b == VPU_PV[0]:
            stage(pv_t, [v_bufs[b][VPU_PV[1], pl.ds(i * 128, 128), :] for i in range(NS)])
    for g, piece in enumerate(WO_PIECES):
        next_piece()
        x = x + _dot(get_o(g).astype(BF), wo.first_read(piece))
        stage_weight(wo, VPU_WO, wo_t, piece)

    y = _with_ones(_layernorm(_layernorm(x)))
    h = None
    for piece in W1_PIECES:
        next_piece()
        d = _dot(_blk(y, *piece[:2]), w1.first_read(piece))
        h = d if h is None else h + d
    w1_sum[...] = h[B:]
    h = _gelu(h[:B] + b1).astype(BF)
    x = x + b2

    def finish_columns(group):
        _, _, j, nj = group[0]
        xj = _blk(x, j, nj)
        for piece in group:
            next_piece()
            xj = xj + _dot(_blk(h, *piece[:2]), w2.first_read(piece))
            stage_weight(w2, VPU_W2, w2_t, piece)
        return j, nj, xj.astype(BF)

    early = []
    for group in W2_GROUPS[:-1]:
        j, nj, xj = finish_columns(group)

        def q_share(i, carry, j=j, nj=nj, xj=xj):
            half = pl.ds(pl.multiple_of(i * (HQ * DH // 2), 128), HQ * DH // 2)
            d = _dot(xj, pltpu.bitcast(wq_packed[WQ_PIECES.index((j, nj, 0, HQ))][:, half], BF))
            q_part[i] = d if j == 0 else q_part[i] + d
            return carry

        lax.fori_loop(0, 2, q_share, None)
        early.append(xj.astype(F32))
    early = _cat(early)
    shift = _mean(early)
    c = early - shift
    sum1, sum2 = jnp.sum(c, axis=-1, keepdims=True), jnp.sum(c * c, axis=-1, keepdims=True)
    j, nj, late = finish_columns(W2_GROUPS[-1])
    assert len(landed) == len(copies)
    c = late.astype(F32) - shift
    dm = (sum1 + jnp.sum(c, axis=-1, keepdims=True)) * (1.0 / D)
    var = (sum2 + jnp.sum(c * c, axis=-1, keepdims=True)) * (1.0 / D) - dm * dm
    mean, mul = shift + dm, lax.rsqrt(jnp.maximum(var, 0.0) + EPS) * q_scale
    x = _cat([early, late.astype(F32)])

    never = zeros[...] != 0
    diagonal = (lax.broadcasted_iota(jnp.int32, (B, 128), 1)
                - lax.broadcasted_iota(jnp.int32, (B, 128), 0)) & 127
    chains = [None] * VPU_CHAINS

    def vpu_matmul(a, wt):
        out = jnp.zeros((B, 128), F32)
        for s in range(128):
            t = _blk(a, 0) * wt[0, pl.ds(s, 8), :]
            if chains[s % VPU_CHAINS] is not None:
                t = jnp.where(never, chains[s % VPU_CHAINS], t)
            for i in range(1, wt.shape[0]):
                t = t + _blk(a, i) * wt[i, pl.ds(s, 8), :]
            chains[s % VPU_CHAINS] = t
            out = jnp.where(diagonal == s, jnp.sum(t, axis=-1, keepdims=True), out)
        return out

    def add_matmul(x, blocks, w, jobs, staged, step):
        acc = [_blk(x, j) for j in range(ND)]
        for k in range(0, len(blocks), step):
            js = [j for j in range(ND) if not any(k0 <= k < k0 + nk and j == j0 for k0, nk, j0 in jobs)]
            d = _dot(_cat(blocks[k:k + step]).astype(BF), w.block(k, step, js))
            for i, j in enumerate(js):
                acc[j] = acc[j] + _blk(d, i)
        for (k, nk, j), wt in zip(jobs, staged):
            assert k % step == 0 and nk % step == 0
            acc[j] = acc[j] + vpu_matmul(_cat(blocks[k:k + nk]), wt)
        return _cat(acc)

    for g in range(HKV):
        q = q_part[g // 2, :, pl.ds(g % 2 * GW, GW)] + _dot(late, wq.block(j, nj, range(g * REP, (g + 1) * REP)))
        put_q(g, (q - mean * wq_sum[:, pl.ds(g * GW, GW)]) * mul)
    pairs = [(b, g) for g in range(HKV) for b in range(B)]
    s, top, p = {}, {}, {}
    for i in range(len(pairs) + LAGS[2]):
        now, at_max, at_exp, at_pv = (pairs[i - n] if 0 <= i - n < len(pairs) else None for n in (0,) + LAGS)
        if now:
            s[now] = logits(*now)
        if at_max:
            top[at_max] = row_max(s[at_max])
        if at_exp:
            p[at_exp] = softmax(s[at_exp], top[at_exp])
        if at_pv == VPU_PV:
            put_o(*at_pv, vpu_matmul(p[at_pv], pv_t))
        elif at_pv:
            put_o(*at_pv, _dot(p[at_pv].astype(BF), pltpu.bitcast(v_packed[at_pv], BF)))
    o = [get_o(g) for g in range(HKV)]
    x = add_matmul(x, [_blk(o[i // REP], i % REP) for i in range(HQ)], wo, VPU_WO, wo_t, STEP_WO)

    xr = x.astype(BF)
    m1, c, r1 = _moments(xr.astype(F32))
    m2, _, r2 = _moments(c * r1)
    mul, sub = r1 * r2, (m1 * r1 + m2) * r2
    h = [_gelu(_dot(xr, w1.column(0, ND, f)) * mul - sub * w1_sum[:, pl.ds(f * 128, 128)] + _blk(b1, f))
         for f in range(NF)]
    x = add_matmul(x + b2, h, w2, VPU_W2, w2_t, STEP_W2)

    out_buf[...] = x.astype(out_buf.dtype)
    copy_out = pltpu.make_async_copy(out_buf, out_hbm, sems.at[0])
    copy_out.start()
    copy_out.wait()


@jax.jit
def pallas_interleave_layers__sliding_block_cached__mixer_channel_mlp__decode_kernel(
    A_x: jax.Array,
    A_k_cache: jax.Array,
    A_v_cache: jax.Array,
    A_wq: jax.Array,
    A_wo: jax.Array,
    B_x: jax.Array,
    B_w1: jax.Array,
    B_b1: jax.Array,
    B_w2: jax.Array,
    B_b2: jax.Array,
):
    del B_x
    sk = A_k_cache.shape[2]
    assert A_x.shape == (B, 1, D) and A_k_cache.shape == A_v_cache.shape == (B, HKV, sk, DH)
    assert min(4096, max(256, sk // 4)) == W and B_w1.shape == (D, F)
    staged = lambda nk: pltpu.VMEM((nk, 136, 128), F32)
    out = pl.pallas_call(
        _kernel,
        out_shape=jax.ShapeDtypeStruct((B, D), A_x.dtype),
        in_specs=[pl.BlockSpec(memory_space=pl.ANY)] * 9,
        out_specs=pl.BlockSpec(memory_space=pl.ANY),
        scratch_shapes=[
            pltpu.VMEM((B, D), BF),
            pltpu.VMEM((NF, 128), BF),
            pltpu.VMEM((ND, 128), BF),
            pltpu.VMEM((B, D), A_x.dtype),
            [pltpu.VMEM((HKV, W, DH), BF)] * B,
            [pltpu.VMEM((HKV, W, DH), BF)] * B,
            _landing_scratch(WQ_PIECES),
            _landing_scratch(WO_PIECES),
            _landing_scratch(W1_PIECES),
            _landing_scratch(W2_PIECES),
            pltpu.VMEM((B, HKV, NS, DH // 2, 128), U32),
            pltpu.VMEM((B, HKV, W // 2, DH), U32),
            _packed_scratch(WQ_PIECES),
            _packed_scratch(WO_PIECES),
            _packed_scratch(W1_PIECES),
            _packed_scratch(W2_PIECES),
            [pltpu.VMEM((REP * B, DH), F32)] * HKV,
            [pltpu.VMEM((B * REP, DH), F32)] * HKV,
            pltpu.VMEM((B, HKV, REP, W), F32),
            pltpu.VMEM((B, HQ * DH), F32),
            pltpu.VMEM((B, F), F32),
            pltpu.VMEM((2, B, HQ * DH // 2), F32),
            staged(NS),
            [staged(nk) for _, nk, _ in VPU_WO],
            [staged(nk) for _, nk, _ in VPU_W2],
            pltpu.VMEM((B, 128), jnp.int32),
            pltpu.SemaphoreType.DMA((IN_FLIGHT,)),
        ],
        compiler_params=pltpu.CompilerParams(vmem_limit_bytes=110 * 1024 * 1024),
    )(
        A_x.reshape(B, D), A_k_cache, A_v_cache, A_wq, A_wo, B_w1,
        B_b1.reshape(NF, 128), B_w2, B_b2.reshape(ND, 128),
    )
    return out.reshape(A_x.shape)
```
